```python
import jax
import jax.numpy as jnp

def _softmax(x, axis=-1):
    return jax.nn.softmax(x, axis=axis)

def _gelu(x):
    return jax.nn.gelu(x, approximate=True)

def _silu(x):
    return jax.nn.silu(x)

def _sigmoid(x):
    return jax.nn.sigmoid(x)

def _layernorm(x, axis=-1, eps=1e-05):
    m = jnp.mean(x, axis=axis, keepdims=True)
    v = jnp.var(x, axis=axis, keepdims=True)
    return (x - m) / jnp.sqrt(v + eps)

def _scatter_add(tgt, idx, src, axis=0):
    return tgt.at[idx].add(src)

def _segment_sum(src, seg, n):
    return jax.ops.segment_sum(src, seg, n)

class _Rng:

    def __init__(self, key):
        self._k = key

    def _next(self):
        self._k, sub = jax.random.split(self._k)
        return sub

    def normal(self, shape):
        return jax.random.normal(self._next(), shape, dtype=jnp.bfloat16)

    def randint(self, lo, hi, shape):
        return jax.random.randint(self._next(), shape, lo, hi, dtype=jnp.int32)

    def uniform(self, shape, lo=0.0, hi=1.0):
        return jax.random.uniform(self._next(), shape, jnp.bfloat16, lo, hi)

    def permutation(self, n):
        return jax.random.permutation(self._next(), n)
kernel_name = 'standalone__conformer_conv_module__speech'

def setup_inputs():
    _rng = _Rng(jax.random.key(int.from_bytes(__import__("os").urandom(4), "little")))
    _w = lambda a: (lambda t: t.astype(jnp.bfloat16) if jnp.issubdtype(t.dtype, jnp.floating) else t)(jnp.asarray(a))
    B, T, D, K = (2, 16000, 256, 31)
    return {'x': _w((lambda *s: _rng.normal(s) * 0.05)(B, T, D)), 'w_pw1': _w((lambda *s: _rng.normal(s) * 0.05)(D, 2 * D)), 'dw': _w((lambda *s: _rng.normal(s) * 0.05)(K, D)), 'w_pw2': _w((lambda *s: _rng.normal(s) * 0.05)(D, D))}

def reference(x, w_pw1, dw, w_pw2):
    B, T, D = x.shape
    K = dw.shape[0]
    h = x @ w_pw1
    a, b = (h[..., :D].copy(), h[..., D:].copy())
    h = a * _sigmoid(b)
    pad = K // 2
    hp = jnp.pad(h, ((0, 0), (pad, pad), (0, 0)))
    out = jnp.zeros_like(h)
    for i in range(K):
        out = out + hp[:, i:i + T, :] * dw[i][None, None, :]
    return _silu(out) @ w_pw2
```

```python
import functools

import jax
import jax.numpy as jnp
import jax.experimental.pallas as pl
import jax.experimental.pallas.tpu as pltpu


def _kernel(xp_ref, x_ref, xn_ref, w1_ref, dw_ref, w2_ref, o_ref, h_ref, *, tb, k):
    j = pl.program_id(1)
    nj = pl.num_programs(1)
    d = x_ref.shape[-1]
    pad = k // 2
    w1 = w1_ref[...]

    def glu(xv):
        h = jnp.dot(xv, w1, preferred_element_type=jnp.float32)
        return h[:, :d] * jax.nn.sigmoid(h[:, d:])

    h_ref[0:16, :] = jnp.where(j > 0, glu(xp_ref[...]), 0.0)
    h_ref[16:16 + tb, :] = glu(x_ref[...])
    h_ref[16 + tb:32 + tb, :] = jnp.where(j < nj - 1, glu(xn_ref[...]), 0.0)
    dw = dw_ref[...].astype(jnp.float32)
    acc = jnp.zeros((tb, d), jnp.float32)
    for i in range(k):
        acc = acc + h_ref[16 - pad + i:16 - pad + i + tb, :] * dw[i:i + 1, :]
    s = acc * jax.nn.sigmoid(acc)
    o_ref[...] = jnp.dot(s.astype(jnp.bfloat16), w2_ref[...],
                         preferred_element_type=jnp.float32).astype(o_ref.dtype)


@jax.jit
def pallas_standalone__conformer_conv_module__speech_kernel(
    x: jax.Array,
    w_pw1: jax.Array,
    dw: jax.Array,
    w_pw2: jax.Array,
):
    b, t, d = x.shape
    k = dw.shape[0]
    tb = 400
    nt = t // tb
    r = tb // 16
    return pl.pallas_call(
        functools.partial(_kernel, tb=tb, k=k),
        grid=(b, nt),
        in_specs=[
            pl.BlockSpec((None, 16, d), lambda i, j: (i, jnp.maximum(j * r - 1, 0), 0)),
            pl.BlockSpec((None, tb, d), lambda i, j: (i, j, 0)),
            pl.BlockSpec((None, 16, d), lambda i, j: (i, jnp.minimum((j + 1) * r, t // 16 - 1), 0)),
            pl.BlockSpec((d, 2 * d), lambda i, j: (0, 0)),
            pl.BlockSpec((k, d), lambda i, j: (0, 0)),
            pl.BlockSpec((d, d), lambda i, j: (0, 0)),
        ],
        out_specs=pl.BlockSpec((None, tb, d), lambda i, j: (i, j, 0)),
        out_shape=jax.ShapeDtypeStruct((b, t, d), x.dtype),
        scratch_shapes=[pltpu.VMEM((tb + 32, d), jnp.float32)],
        compiler_params=pltpu.CompilerParams(
            dimension_semantics=("parallel", "parallel")),
    )(x, x, x, w_pw1, dw, w_pw2)
```

```python
import functools
import jax
import jax.numpy as jnp
import jax.experimental.pallas as pl
import jax.experimental.pallas.tpu as pltpu

F32, BF16, I32 = jnp.float32, jnp.bfloat16, jnp.int32
HALO = 16


def _add(a, b):
    return b if a is None else a if b is None else a + b


def _split_w(w, lv):
    if lv == 0:
        return [w]
    w0, w1 = w[0::2], w[1::2]
    return (_split_w([_add(a, b) for a, b in zip(w0, w1)], lv - 1)
            + _split_w(w0, lv - 1) + _split_w(w1, lv - 1))


def _pre(x, lv):
    if lv == 0:
        return [x]
    x = functools.lru_cache(None)(x)
    return (_pre(lambda m: x(2 * m + 1), lv - 1)
            + _pre(lambda m: x(2 * m) - x(2 * m + 1), lv - 1)
            + _pre(lambda m: x(2 * m + 2) - x(2 * m + 1), lv - 1))


def _post(sub, lv, base, n):
    if lv == 0:
        return sub(base, n)
    st = 3 ** (lv - 1)
    m1 = _post(sub, lv - 1, base, n // 2)
    y0 = [a + b for a, b in zip(m1, _post(sub, lv - 1, base + st, n // 2))]
    y1 = [a + b for a, b in zip(m1, _post(sub, lv - 1, base + 2 * st, n // 2))]
    return [v for p in zip(y0, y1) for v in p]


def _kernel(x_ref, w1_ref, dw_ref, w2_ref, o_ref,
            h_ref, y_ref, p_ref, wc_ref, w1s, w2s, *, seg, lv, grp, bpb, k, nb, ma, md, zero, pd):
    g = pl.program_id(0)
    d = x_ref.shape[-1]
    nl = d // 128
    tb = 8 * seg
    par = 2 ** lv
    taps = 32 // par
    ng = seg // par
    struct = _split_w([None] * (32 - k) + [0] * k, lv)

    @pl.when(g == 0)
    def _():
        for l in range(nl):
            w1s[l] = pltpu.bitcast(w1_ref[:, l * 128:(l + 1) * 128], I32)
            w1s[nl + l] = pltpu.bitcast((w1_ref[:, d + l * 128:d + (l + 1) * 128].astype(F32) * 0.5).astype(BF16), I32)
            w2s[l] = pltpu.bitcast(w2_ref[:, l * 128:(l + 1) * 128], I32)
        dwv = dw_ref[...].astype(F32) * 0.25
        for l in range(nl):
            w = [None] * (32 - k) + [dwv[i:i + 1, l * 128:(l + 1) * 128] for i in range(k)]
            for s, ws in enumerate(_split_w(w, lv)):
                for j, v in enumerate(ws):
                    if v is not None:
                        wc_ref[l, s * taps + j] = jnp.broadcast_to(v, (8, 128))
        h_ref[1] = jnp.zeros_like(h_ref[1]); h_ref[0, :, 0:HALO] = jnp.zeros((nl, HALO, 128), F32)
        y_ref[1] = jnp.zeros_like(y_ref[1])

    def stage_a(sa, xoff, r0):
        xv = x_ref[pl.ds(xoff + r0, ma), :]
        w = jnp.concatenate([pltpu.bitcast(w1s[i], BF16) for i in range(2 * nl)], axis=1)
        h = jnp.dot(xv, w, preferred_element_type=F32)
        for l in range(nl):
            a = h[:, l * 128:(l + 1) * 128]
            h_ref[sa, l, pl.ds(HALO + r0, ma)] = a * (1.0 + jnp.tanh(h[:, d + l * 128:d + (l + 1) * 128]))

    def stage_b(sa, l, m0, n):
        seqs = _pre(lambda i: h_ref[1 - sa, l, pl.ds(m0 * par + i, 8, stride=seg), :], lv)
        for m in range(n):
            for s, f in enumerate(seqs):
                p_ref[(sa if pd else 0), l, s, m0 + m] = f(m)

    def stage_c(sa, l, m0, grp, hook):
        def sub(s, n):
            acc = [None] * n
            xs = [p_ref[(sa if pd else 0), l, s, m0 + i] for i in range(n + taps - 1)]
            for j in range(taps):
                if struct[s][j] is None:
                    continue
                w = wc_ref[l, s * taps + j]
                for i in range(n):
                    acc[i] = _add(acc[i], xs[i + j] * w)
            hook(n)
            return acc
        for i, u in enumerate(_post(sub, lv, 0, grp * par)):
            y_ref[sa, l, pl.ds(m0 * par + i, 8, stride=seg), :] = u + u * jnp.tanh(u)

    def stage_d(sa, ooff, r0):
        s = jnp.concatenate([y_ref[1 - sa, l, pl.ds(r0, md)] for l in range(nl)], axis=1).astype(BF16)
        w = jnp.concatenate([pltpu.bitcast(w2s[i], BF16) for i in range(nl)], axis=1)
        o_ref[pl.ds(ooff + r0, md), :] = jnp.dot(s, w, preferred_element_type=F32).astype(o_ref.dtype)

    lead = taps - 1 + grp
    def block(q, _):
        blk = g * nb + q
        sa = blk % 2
        off = pl.multiple_of(q * tb, 16)
        tasks = sorted([(r, 1, 2 * ma) for r in range(0, tb, ma)] + [(r, 0, md) for r in range(0, tb, md)])
        st = [0, 0, 0]
        def hook(n):
            st[0] += n
            while st[1] < len(tasks) and st[2] * nl * 3 ** lv * ng <= st[0] * 3 * tb:
                r, isa, cost = tasks[st[1]]
                (stage_a if isa else stage_d)(sa, off, r)
                if isa and r == 0:
                    h_ref[1 - sa, :, HALO + tb:] = jnp.where(blk % bpb != 0, h_ref[sa, :, HALO:2 * HALO], 0.0)
                st[1] += 1
                st[2] += cost
        for l in range(nl):
            for m in range(0, lead, grp):
                hook(0)
                st[0] += zero
                stage_b(sa, l, m, min(grp, lead - m))
        for m0 in range(0, ng, grp):
            for l in range(nl):
                n = min(grp, ng + taps - 1 - m0 - lead)
                if n > 0:
                    stage_b(sa, l, m0 + lead, n)
                stage_c(sa, l, m0, min(grp, ng - m0), hook)
        assert st[1] == len(tasks)
        h_ref[1 - sa, :, 0:HALO] = jnp.where(blk % bpb != bpb - 1, h_ref[sa, :, tb:tb + HALO], 0.0)
    jax.lax.fori_loop(0, nb, block, None)


def _run(x, w_pw1, dw, w_pw2, seg=100, lv=2, grp=3, nb=2, ma=80, md=80, zero=1, pd=1):
    b, t, d = x.shape
    k = dw.shape[0]
    tb = 8 * seg
    n = b * t // (nb * tb)
    nl = d // 128
    par = 2 ** lv
    out = pl.pallas_call(
        functools.partial(_kernel, seg=seg, lv=lv, grp=grp, bpb=t // tb, k=k, nb=nb, ma=ma, md=md, zero=zero, pd=pd),
        grid=(n + 2 // nb,),
        in_specs=[
            pl.BlockSpec((nb * tb, d), lambda g: (jnp.minimum(g, n - 1), 0)),
            pl.BlockSpec((d, 2 * d), lambda g: (0, 0)),
            pl.BlockSpec((k, d), lambda g: (0, 0)),
            pl.BlockSpec((d, d), lambda g: (0, 0)),
        ],
        out_specs=pl.BlockSpec((nb * tb, d), lambda g: (jnp.maximum(g - 2 // nb, 0), 0)),
        out_shape=jax.ShapeDtypeStruct((b * t, d), x.dtype),
        scratch_shapes=[
            pltpu.VMEM((2, nl, tb + 2 * HALO, 128), F32),
            pltpu.VMEM((2, nl, tb, 128), F32),
            pltpu.VMEM((2, nl, 3 ** lv, (seg + 32) // par, 8, 128), F32),
            pltpu.VMEM((nl, 3 ** lv * 32 // par, 8, 128), F32),
            pltpu.VMEM((2 * nl, d // 2, 128), I32),
            pltpu.VMEM((nl, d // 2, 128), I32),
        ],
        compiler_params=pltpu.CompilerParams(vmem_limit_bytes=100<<20, dimension_semantics=("arbitrary",)),
        name="conformer_kernel",
    )(x.reshape(b * t, d), w_pw1, dw, w_pw2)
    return out.reshape(b, t, d)


@jax.jit
def pallas_standalone__conformer_conv_module__speech_kernel(x, w_pw1, dw, w_pw2):
    return _run(x, w_pw1, dw, w_pw2)
```
